```python
import jax
import jax.numpy as jnp

def _softmax(x, axis=-1):
    return jax.nn.softmax(x, axis=axis)
def _gelu(x):
    return jax.nn.gelu(x, approximate=True)
def _silu(x):
    return jax.nn.silu(x)
def _sigmoid(x):
    return jax.nn.sigmoid(x)
def _layernorm(x, axis=-1, eps=1e-5):
    m = jnp.mean(x, axis=axis, keepdims=True)
    v = jnp.var(x, axis=axis, keepdims=True)
    return (x - m) / jnp.sqrt(v + eps)
def _scatter_add(tgt, idx, src, axis=0):
    return tgt.at[idx].add(src)
def _segment_sum(src, seg, n):
    return jax.ops.segment_sum(src, seg, n)
class _Rng:
    def __init__(self, key):
        self._k = key
    def _next(self):
        self._k, sub = jax.random.split(self._k)
        return sub
    def normal(self, shape):
        return jax.random.normal(self._next(), shape, dtype=jnp.bfloat16)
    def randint(self, lo, hi, shape):
        return jax.random.randint(self._next(), shape, lo, hi, dtype=jnp.int32)
    def uniform(self, shape, lo=0.0, hi=1.0):
        return jax.random.uniform(self._next(), shape, jnp.bfloat16, lo, hi)
    def permutation(self, n):
        return jax.random.permutation(self._next(), n)


kernel_name = 'parallel_sum__compressed_kv_cla__moe_arch_mod__prompt'

def setup_inputs():
    _rng = _Rng(jax.random.key(int.from_bytes(__import__("os").urandom(4), "little")))
    _w = (lambda a: (lambda t: t.astype(jnp.bfloat16) if jnp.issubdtype(t.dtype, jnp.floating) else t)(jnp.asarray(a)))
    def _A_setup():
        B, H, Sq, Sk, D, M = 1, 32, 2048, 2048, 128, 640
        Dc = 4 * D
        return {
            "x": _w((lambda *s: _rng.normal(s) * 0.05)(B, Sq, M)),
            "c_kv": _w((lambda *s: _rng.normal(s) * 0.05)(B, Sk, Dc)),
            "w_q": _w((lambda *s: _rng.normal(s) * 0.05)(M, H, D) * (M ** -0.5)),
            "w_uk": _w((lambda *s: _rng.normal(s) * 0.05)(Dc, H, D) * (Dc ** -0.5)),
            "w_uv": _w((lambda *s: _rng.normal(s) * 0.05)(Dc, H, D) * (Dc ** -0.5)),
            "w_o": _w((lambda *s: _rng.normal(s) * 0.05)(H, D, M) * ((H * D) ** -0.5)),
        }
    _A_in = _A_setup()

    def _B_setup():
        B, S, D, F, C = 1, 2048, 640, 1728, 8
        return {
            "x": _w((lambda *s: _rng.normal(s) * 0.05)(B, S, D)),
            "w_r": _w((lambda *s: _rng.normal(s) * 0.05)(D)),
            "w_gate": _w((lambda *s: _rng.normal(s) * 0.05)(D, F)),
            "w_up": _w((lambda *s: _rng.normal(s) * 0.05)(D, F)),
            "w_down": _w((lambda *s: _rng.normal(s) * 0.05)(F, D)),
        }
    _B_in = _B_setup()

    return {
        "A_x": _A_in["x"],
        "A_c_kv": _A_in["c_kv"],
        "A_w_q": _A_in["w_q"],
        "A_w_uk": _A_in["w_uk"],
        "A_w_uv": _A_in["w_uv"],
        "A_w_o": _A_in["w_o"],
        "B_x": _B_in["x"],
        "B_w_r": _B_in["w_r"],
        "B_w_gate": _B_in["w_gate"],
        "B_w_up": _B_in["w_up"],
        "B_w_down": _B_in["w_down"],
    }

def reference(A_x, A_c_kv, A_w_q, A_w_uk, A_w_uv, A_w_o, B_x, B_w_r, B_w_gate, B_w_up, B_w_down):
    def _A_ref(x, c_kv, w_q, w_uk, w_uv, w_o):
        B, Sq, M = x.shape[0], x.shape[1], x.shape[2]
        Sk = c_kv.shape[1]
        H, D = w_q.shape[1], w_q.shape[2]
        q = jnp.einsum("bqm,mhd->bhqd", x, w_q)
        k = jnp.einsum("bkc,chd->bhkd", c_kv, w_uk)
        v = jnp.einsum("bkc,chd->bhkd", c_kv, w_uv)
        scores = jnp.einsum("bhqd,bhkd->bhqk", q, k) * (D ** -0.5)
        off = Sk - Sq
        qi = jnp.arange(Sq)[:, None]
        kj = jnp.arange(Sk)[None, :]
        cmask = kj <= (qi + off)
        scores = jnp.where(cmask[None, None], scores, -1e9)
        p = _softmax(scores, axis=-1)
        ctx = jnp.einsum("bhqk,bhkd->bhqd", p, v)
        return jnp.einsum("bhqd,hdm->bqm", ctx, w_o)

    def _B_ref(x, w_r, w_gate, w_up, w_down):
        B, S, D = x.shape
        C = 8
        r = x @ w_r
        idx = jnp.argsort(-r, axis=-1)[:, :C]
        idx_e = jnp.repeat(idx.reshape(B, C, 1), D, axis=2)
        x_sel = jnp.take_along_axis(x, idx_e, axis=1)
        g = _silu(x_sel @ w_gate)
        u = x_sel @ w_up
        y = (g * u) @ w_down
        r_sel = _sigmoid(jnp.take_along_axis(r, idx, axis=1))
        y = y * r_sel.reshape(B, C, 1)
        b_off = (jnp.arange(B) * S).reshape(B, 1)
        flat_idx = (idx + b_off).reshape(B * C)
        zero = (x * 0.0).reshape(B * S, D)
        upd = _scatter_add(zero, flat_idx, y.reshape(B * C, D), axis=0)
        return x + upd.reshape(B, S, D)

    x = A_x
    xn = _layernorm(x, axis=-1)
    return x + _A_ref(xn, A_c_kv, A_w_q, A_w_uk, A_w_uv, A_w_o) + _B_ref(xn, B_w_r, B_w_gate, B_w_up, B_w_down)
```

```python
import functools
import numpy as np
import jax
import jax.numpy as jnp
from jax import lax
import jax.experimental.pallas as pl
import jax.experimental.pallas.tpu as pltpu

F32, BF16, I32, U32 = jnp.float32, jnp.bfloat16, jnp.int32, jnp.uint32
NT = (((1,), (1,)), ((), ()))
T = 128
BQ = 512
BK = 512
RB = 256
CAP = 8
LOG2E = float(np.log2(np.e))
SAFE = float(2.0 ** 40)


def _rb(a):
    return a.astype(BF16).astype(F32)


def _dot(a, b):
    return jnp.dot(a, b, preferred_element_type=F32)


def _dot_nt(a, b):
    return lax.dot_general(a, b, NT, preferred_element_type=F32)


def _fold(a):
    parts = [a[:, t:t + T] for t in range(0, a.shape[1], T)]
    s = functools.reduce(jnp.add, parts)
    return jnp.sum(s.reshape(-1, 8, T), axis=0)


def _big(w):
    t = (w & np.uint32(0x7F807F80)) + np.uint32(0x36003600)
    parts = [t[r:r + 8, c:c + T] for r in range(0, t.shape[0], 8) for c in range(0, t.shape[1], T)]
    lanes = [functools.reduce(jnp.bitwise_or, parts[n::4]) for n in range(4)]
    return functools.reduce(jnp.bitwise_or, lanes) & np.uint32(0x80008000)


def _kernel(x_hbm, c_hbm, wq_hbm, wk_hbm, wv_hbm, wo_hbm, wr_ref, wg_hbm, wu_hbm, wd_hbm, o_hbm,
            x_ref, c_ref, xn_ref, acc_ref, ob_ref, q_ref, k_ref, v_ref, ctx_ref,
            wq_s, wk_s, wv_s, wo_ref, wq_b, wk_b, wv_b, wg_ref, wu_ref, wd_ref,
            y_ref, idx_ref, x_sem, w_sem, o_sem, m_sem):
    S, M = x_ref.shape
    HP, _, D = wq_s.shape
    NQ = S // BQ
    qscale = np.float32(D ** -0.5 * LOG2E)

    def x_copy(i):
        return pltpu.make_async_copy(x_hbm.at[pl.ds(i * RB, RB)], x_ref.at[pl.ds(i * RB, RB)], x_sem.at[i])

    def w_copies(j):
        cps = [pltpu.make_async_copy(src.bitcast(U32).at[:, j, :], dst.at[j], w_sem.at[j])
               for src, dst in ((wk_hbm, wk_s), (wq_hbm, wq_s), (wv_hbm, wv_s))]
        return cps + [pltpu.make_async_copy(wo_hbm.at[j], wo_ref.at[j], w_sem.at[j])]

    def o_copy(i):
        return pltpu.make_async_copy(ob_ref.at[pl.ds(i * BQ, BQ)], o_hbm.at[pl.ds(i * BQ, BQ)], o_sem.at[i])

    c_copy = pltpu.make_async_copy(c_hbm, c_ref, m_sem.at[0])
    ffn_copies = [pltpu.make_async_copy(s, d, m_sem.at[1 + n])
                  for n, (s, d) in enumerate(((wg_hbm, wg_ref), (wu_hbm, wu_ref), (wd_hbm, wd_ref)))]

    def unpack(j):
        for src, dst in ((wk_s, wk_b), (wq_s, wq_b), (wv_s, wv_b)):
            w = src[j]
            dst[:, :D] = lax.bitcast_convert_type(w << 16, F32).astype(BF16)
            dst[:, D:] = lax.bitcast_convert_type(w & np.uint32(0xFFFF0000), F32).astype(BF16)

    def residual(rows, x, xn):
        xf = xn.astype(F32)
        acc_ref[rows, :] = x + (xf + xf * 0.0)

    def scatter():
        for c in range(CAP):
            acc_ref[pl.ds(idx_ref[c], 1), :] += y_ref[c:c + 1, :]

    for i in range(S // RB):
        x_copy(i).start()
    c_copy.start()
    for cp in w_copies(0):
        cp.start()

    def ln_body(i, _):
        x_copy(i).wait()
        rows = pl.ds(pl.multiple_of(i * RB, RB), RB)
        x = x_ref[rows, :].astype(F32)
        mean = jnp.sum(x, axis=1, keepdims=True) / M
        cen = x - mean
        var = jnp.sum(cen * cen, axis=1, keepdims=True) / M
        d = _rb(x - _rb(mean))
        sd = _rb(jnp.sqrt(_rb(_rb(var) + np.float32(np.float32(1e-5).astype(BF16)))))
        xn = (d * (1.0 / sd)).astype(BF16)
        xn_ref[rows, :] = xn
        residual(rows, x, xn)
        return 0
    lax.fori_loop(0, S // RB, ln_body, 0)

    for cp in w_copies(1):
        cp.start()

    r = _rb(_dot_nt(jnp.broadcast_to(wr_ref[...].astype(F32), (8, M)).astype(BF16), xn_ref[...]))
    b = lax.shift_right_logical(lax.bitcast_convert_type(r, I32), 16)
    b = jnp.where(b == 0x8000, 0, b)
    key = jnp.where(b >= 0x8000, 0xFFFF - b, b + 0x8000)
    key = jnp.where((b & 0x7FFF) > 0x7F80, 0, key)
    pos = lax.broadcasted_iota(I32, (8, S), 1)
    key = lax.bitcast_convert_type((key * S + (S - 1 - pos)) | (1 << 29), F32)
    sub = lax.broadcasted_iota(I32, (8, 1), 0)
    top = jnp.zeros((8, 1), F32)
    for c in range(CAP):
        mx = jnp.max(key, axis=1, keepdims=True)
        top = jnp.where(sub == c, mx, top)
        key = jnp.where(key == mx, 0.0, key)
    top = lax.bitcast_convert_type(top, I32)
    sel = (S - 1) - (top & (S - 1))
    onehot = (pos == sel)
    r_sel = jnp.sum(jnp.where(onehot, r, 0.0), axis=1, keepdims=True)
    for c in range(CAP):
        idx_ref[c] = sel[c, 0]
    y_ref[...] = jnp.broadcast_to(_rb(jax.nn.sigmoid(r_sel)), (CAP, M))

    def ffn():
        xn32 = xn_ref.bitcast(U32)
        xs = jnp.zeros((CAP, M), U32)
        subm = lax.broadcasted_iota(I32, (CAP, M), 0)
        for c in range(CAP):
            i = idx_ref[c]
            w = xn32[pl.ds(i >> 1, 1), :]
            w = (w >> ((i & 1) * 16).astype(U32)) << 16
            xs = jnp.where(subm == c, w, xs)
        xs = lax.bitcast_convert_type(xs, F32).astype(BF16)
        g = _rb(_dot_nt(xs, wg_ref[...]))
        u = _rb(_dot_nt(xs, wu_ref[...]))
        hid = (_rb(g * jax.nn.sigmoid(g)) * u).astype(BF16)
        y_ref[...] = _rb(_rb(_dot(hid, wd_ref[...])) * y_ref[...])
        scatter()

    c_copy.wait()
    for cp in w_copies(0):
        cp.wait()
    for cp in ffn_copies:
        cp.start()
    unpack(0)

    def out_proj(j, qi):
        rows = slice(qi * BQ, (qi + 1) * BQ)
        a = acc_ref[rows, :] + _dot(ctx_ref[rows, :], wo_ref[j])
        acc_ref[rows, :] = a
        ob_ref[rows, :] = a.astype(BF16)
        pl.when(j == HP - 1)(lambda: o_copy(qi).start())

    def pair_body(j, chk):
        @pl.when(j + 2 < HP)
        def _():
            for cp in w_copies(j + 2):
                cp.start()

        @pl.when(j + 1 < HP)
        def _():
            for cp in w_copies(j + 1):
                cp.wait()

        @pl.when(j == 1)
        def _():
            for cp in ffn_copies:
                cp.wait()
            ffn()


        k_ref[...] = _dot(c_ref[...], wk_b[...]).astype(BF16)
        for r0 in range(0, S, S // 2):
            rows = slice(r0, r0 + S // 2)
            q_ref[rows, :] = (_dot(xn_ref[rows, :], wq_b[...]) * qscale).astype(BF16)
        v_ref[...] = _dot(c_ref[...], wv_b[...]).astype(BF16)
        unpack(jnp.minimum(j + 1, HP - 1))

        tri = lax.broadcasted_iota(I32, (T, T), 1) <= lax.broadcasted_iota(I32, (T, T), 0)
        nt = BQ // T
        for qi in range(NQ):
            q0 = qi * BQ
            for h in range(2):
                hs = slice(h * D, (h + 1) * D)
                q = q_ref[q0:q0 + BQ, hs]
                ps = []
                for t in range(nt):
                    k0 = q0 + t * T
                    p = jnp.exp2(_dot_nt(q[t * T:], k_ref[k0:k0 + T, hs]))
                    pd = jnp.where(tri, p[:T], 0.0)
                    ps.append(jnp.concatenate([pd, p[T:]], axis=0) if t < nt - 1 else pd)
                accs, ls = [None] * nt, [None] * nt
                for t in range(nt):
                    k0 = q0 + t * T
                    o = _dot(ps[t].astype(BF16), v_ref[k0:k0 + T, hs])
                    for u in range(t, nt):
                        sl = slice((u - t) * T, (u - t + 1) * T)
                        ls[u] = ps[t][sl] if t == 0 else ls[u] + ps[t][sl]
                        accs[u] = o[sl] if t == 0 else accs[u] + o[sl]
                acc = jnp.concatenate(accs, axis=0)
                l = jnp.concatenate(ls, axis=0)
                for k0 in range(0, q0, BK):
                    p = jnp.exp2(_dot_nt(q, k_ref[k0:k0 + BK, hs]))
                    for t in range(0, BK, T):
                        l = l + p[:, t:t + T]
                    acc = acc + _dot(p.astype(BF16), v_ref[k0:k0 + BK, hs])
                l = jnp.sum(l, axis=1, keepdims=True)
                rl = pl.reciprocal(l, approx=True)
                rl = rl * (2.0 - l * rl)
                ctx_ref[q0:q0 + BQ, hs] = (acc * rl).astype(BF16)
                chk = chk + jnp.sum((l + rl).reshape(-1, 8, 1), axis=0)
                if h == 0 and qi == 2:
                    out_proj(j, 0)
                    out_proj(j, 1)
        out_proj(j, 2)
        out_proj(j, 3)
        return chk

    chk = lax.fori_loop(0, HP, pair_body, jnp.zeros((8, T), F32))
    big = functools.reduce(jnp.bitwise_or, [_big(c_ref.bitcast(U32)[...])] + [_big(wv_s[j]) for j in range(HP)])
    unsafe = jnp.max(jnp.where((chk < SAFE) & (big == 0), 0.0, 1.0)) > 0.0
    for qi in range(NQ):
        o_copy(qi).wait()

    @pl.when(unsafe)
    def _():
        def blocks(body):
            def step(i, _):
                body(i, pl.ds(pl.multiple_of(i * RB, RB), RB))
                return 0
            lax.fori_loop(0, S // RB, step, 0)

        blocks(lambda i, rows: residual(rows, x_ref[rows, :].astype(F32), xn_ref[rows, :]))
        scatter()

        def pair(j, _):
            unpack(j)

            def proj(i, rows):
                q_ref[rows, :] = (_dot(xn_ref[rows, :], wq_b[...]) * qscale).astype(BF16)
                k_ref[rows, :] = _dot(c_ref[rows, :], wk_b[...]).astype(BF16)
                v_ref[rows, :] = _dot(c_ref[rows, :], wv_b[...]).astype(BF16)
            blocks(proj)

            def attend(i, rows):
                keep = (lax.broadcasted_iota(I32, (RB, S), 1)
                        <= lax.broadcasted_iota(I32, (RB, S), 0) + i * RB)
                for h in range(2):
                    hs = slice(h * D, (h + 1) * D)
                    s = jnp.where(keep, _dot_nt(q_ref[rows, hs], k_ref[:, hs]), np.float32(-1e9 * LOG2E))
                    p = jnp.exp2(s - jnp.max(s, axis=1, keepdims=True))
                    p = p / jnp.sum(p, axis=1, keepdims=True)
                    ctx_ref[rows, hs] = _dot(p.astype(BF16), v_ref[:, hs]).astype(BF16)
                acc_ref[rows, :] += _dot(ctx_ref[rows, :], wo_ref[j])
            blocks(attend)
            return 0
        lax.fori_loop(0, HP, pair, 0)

        def fin(i, rows):
            ob_ref[rows, :] = acc_ref[rows, :].astype(BF16)
        blocks(fin)
        for qi in range(NQ):
            o_copy(qi).start()
        for qi in range(NQ):
            o_copy(qi).wait()


@jax.jit
def pallas_parallel_sum__compressed_kv_cla__moe_arch_mod__prompt_kernel(
        A_x, A_c_kv, A_w_q, A_w_uk, A_w_uv, A_w_o, B_x, B_w_r, B_w_gate, B_w_up, B_w_down):
    _, S, M = A_x.shape
    DC = A_c_kv.shape[2]
    _, H, D = A_w_q.shape
    F = B_w_down.shape[0]
    HP = H // 2
    vm = pltpu.VMEM
    hbm = pl.BlockSpec(memory_space=pl.ANY)
    out = pl.pallas_call(
        _kernel,
        out_shape=jax.ShapeDtypeStruct((S, M), BF16),
        in_specs=[hbm] * 6 + [pl.BlockSpec(memory_space=vm)] + [hbm] * 3,
        out_specs=hbm,
        scratch_shapes=[
            vm((S, M), BF16), vm((S, DC), BF16), vm((S, M), BF16), vm((S, M), F32), vm((S, M), BF16),
            vm((S, 2 * D), BF16), vm((S, 2 * D), BF16), vm((S, 2 * D), BF16), vm((S, 2 * D), BF16),
            vm((HP, M, D), U32), vm((HP, DC, D), U32), vm((HP, DC, D), U32), vm((HP, 2 * D, M), BF16),
            vm((M, 2 * D), BF16), vm((DC, 2 * D), BF16), vm((DC, 2 * D), BF16),
            vm((F, M), BF16), vm((F, M), BF16), vm((F, M), BF16),
            vm((CAP, M), F32), pltpu.SMEM((CAP,), I32),
            pltpu.SemaphoreType.DMA((S // RB,)), pltpu.SemaphoreType.DMA((HP,)),
            pltpu.SemaphoreType.DMA((S // BQ,)), pltpu.SemaphoreType.DMA((4,)),
        ],
        compiler_params=pltpu.CompilerParams(vmem_limit_bytes=100 * 1024 * 1024),
    )(A_x.reshape(S, M), A_c_kv.reshape(S, DC), A_w_q, A_w_uk, A_w_uv, A_w_o.reshape(HP, 2 * D, M),
      B_w_r.reshape(1, M), B_w_gate.T, B_w_up.T, B_w_down)
    return out.reshape(1, S, M)
```

```python
import functools
import numpy as np
import jax
import jax.numpy as jnp
from jax import lax
import jax.experimental.pallas as pl
import jax.experimental.pallas.tpu as pltpu

F32, BF16, I32, U32 = jnp.float32, jnp.bfloat16, jnp.int32, jnp.uint32
NT = (((1,), (1,)), ((), ()))
T = 128
BQ = 512
BK = 512
RB = 256
LB = 64
PLAN = (0, 0, 1, 1, 0, 1, 0, 1)
AHEAD = 2
OB = (0, 512, 1024, 1536, 1792, 2048)
CAP = 8
LOG2E = float(np.log2(np.e))
SAFE = float(2.0 ** 40)
EPS = np.float32(np.float32(1e-5).astype(BF16))
MASKED = np.float32(float(np.float32(-1e9).astype(BF16)) * LOG2E)


def _rb(a):
    return a.astype(BF16).astype(F32)


def _dot(a, b):
    return jnp.dot(a, b, preferred_element_type=F32)


def _dot_nt(a, b):
    return lax.dot_general(a, b, NT, preferred_element_type=F32)


def _half(w, h):
    w = (w << 16) if h == 0 else (w & np.uint32(0xFFFF0000))
    return lax.bitcast_convert_type(w, F32).astype(BF16)


def _big(w):
    t = (w & np.uint32(0x7F807F80)) + np.uint32(0x36003600)
    parts = [t[r:r + 8, c:c + T] for r in range(0, t.shape[0], 8) for c in range(0, t.shape[1], T)]
    return functools.reduce(jnp.bitwise_or, parts) & np.uint32(0x80008000)


def _kernel(x_hbm, c_hbm, wq_hbm, wk_hbm, wv_hbm, wo_hbm, wr_ref, wg_hbm, wu_hbm, wd_hbm, o_hbm,
            x_ref, c_ref, xn_ref, acc_ref, ob_ref, q_ref, k_ref, v_ref, ctx_ref,
            wq_s, wk_s, wv_s, wo_ref, wq_b, wk_b, wv_b, wg_ref, wu_ref, wd_ref,
            r_ref, sel_ref, gate_ref, xs_ref, y_ref, idx_ref, in_sem, w_sem, o_sem, m_sem):
    S, M = x_ref.shape
    HP, _, D = wq_s.shape
    F = wd_ref.shape[0]
    NQ, NB = S // BQ, S // RB
    qscale = np.float32(D ** -0.5 * LOG2E)

    def in_copies(i):
        rows = pl.ds(i * RB, RB)
        return [pltpu.make_async_copy(s.at[rows], d.at[rows], in_sem.at[i])
                for s, d in ((c_hbm, c_ref), (x_hbm, x_ref))]

    def pair_copy(src, dst, j, sem):
        return pltpu.make_async_copy(src.bitcast(U32).at[:, j, :], dst.at[j], sem)

    def kv_copies(j, sem):
        return [pair_copy(wk_hbm, wk_s, j, sem), pair_copy(wv_hbm, wv_s, j, sem)]

    def qo_copies(j, sem):
        return [pair_copy(wq_hbm, wq_s, j, sem), pltpu.make_async_copy(wo_hbm.at[j], wo_ref.at[j], sem)]

    def w_copies(j):
        return kv_copies(j, w_sem.at[j]) + qo_copies(j, w_sem.at[j])

    def o_copy(n):
        rows = pl.ds(OB[n], OB[n + 1] - OB[n])
        return pltpu.make_async_copy(ob_ref.at[rows], o_hbm.at[rows], o_sem.at[n])

    def start(cps):
        for cp in cps:
            cp.start()

    def wait(cps):
        for cp in cps:
            cp.wait()

    kv01 = kv_copies(0, m_sem.at[0]) + kv_copies(1, m_sem.at[0])
    qo01 = qo_copies(0, m_sem.at[1]) + qo_copies(1, m_sem.at[1])
    ffn_copies = [pltpu.make_async_copy(s, d, m_sem.at[2])
                  for s, d in ((wg_hbm, wg_ref), (wu_hbm, wu_ref), (wd_hbm, wd_ref))]

    def unpack(src, dst):
        w = src[...]
        for h in range(2):
            dst[h] = _half(w, h)

    def finish(rows, a):
        xn = xn_ref[rows, :].astype(F32)
        ob_ref[rows, :] = (a + (x_ref[rows, :].astype(F32) + (xn + xn * 0.0))).astype(BF16)

    def scatter():
        y = _rb(_rb(y_ref[...]) * gate_ref[...])
        for c in range(CAP):
            acc_ref[pl.ds(idx_ref[c], 1), :] += y[c:c + 1, :]

    start(kv01)
    start(in_copies(0))
    wr = wr_ref[...].astype(F32).reshape(1, M)
    diag = lax.broadcasted_iota(I32, (T, T), 0) == lax.broadcasted_iota(I32, (T, T), 1)
    wait(kv01)
    for i in range(1, AHEAD):
        start(in_copies(i))
    for n in range(2):
        unpack(wk_s.at[n], wk_b.at[n])
        unpack(wv_s.at[n], wv_b.at[n])

    def norm_rows(r0):
        rows = pl.ds(pl.multiple_of(r0, LB), LB)
        x = x_ref[rows, :].astype(F32)
        mean = jnp.sum(x, axis=1, keepdims=True) / M
        cen = x - mean
        var = jnp.sum(cen * cen, axis=1, keepdims=True) / M
        d = _rb(x - _rb(mean))
        sd = _rb(jnp.sqrt(_rb(_rb(var) + EPS)))
        xn = (d * (1.0 / sd)).astype(BF16)
        xn_ref[rows, :] = xn
        acc_ref[rows, :] = jnp.zeros((LB, M), F32)
        return jnp.sum(xn.astype(F32) * wr, axis=1, keepdims=True)

    def first_rows(i, _):
        pl.when(i + AHEAD < NB)(lambda: start(in_copies(i + AHEAD)))
        pl.when(i == NB // 2)(lambda: start(qo01))
        wait(in_copies(i))
        rows = pl.ds(pl.multiple_of(i * RB, RB), RB)
        c = c_ref[rows, :]
        zero = i >> 20
        todo = list(range(0, RB, LB))
        racc = [None] * (RB // T)
        for g in range(8):
            n, h = g // 4, g // 2 % 2
            dep = None
            for _k in range(PLAN[g]):
                p0 = todo.pop(0)
                r = jnp.where(diag[p0 % T:p0 % T + LB], norm_rows(i * RB + p0), 0.0)
                r = jnp.sum(r.reshape(-1, 8, T), axis=0)
                racc[p0 // T] = r if racc[p0 // T] is None else racc[p0 // T] + r
                dep = r if dep is None else dep + r
            cg = c
            if dep is not None:
                z = lax.bitcast_convert_type(dep, I32) & zero
                head = pltpu.bitcast(c[:16], I32) | jnp.concatenate([z] * (c.shape[1] // T), axis=1)
                cg = jnp.concatenate([pltpu.bitcast(head, BF16), c[16:]], axis=0)
            dst, w = (k_ref, wk_b) if g % 2 == 0 else (v_ref, wv_b)
            dst[n, h, rows, :] = _dot(cg, w[n, h]).astype(BF16)
        for t in range(RB // T):
            r_ref[pl.ds(i * (RB // T) + t, 1), :] = jnp.sum(racc[t], axis=0, keepdims=True)
        return 0
    lax.fori_loop(0, NB, first_rows, 0)
    wait(qo01)
    start(ffn_copies)
    unpack(wq_s.at[0], wq_b.at[0])

    def top_tokens():
        b = lax.shift_right_logical(lax.bitcast_convert_type(_rb(r_ref[...]), I32), 16)
        b = jnp.where(b == 0x8000, 0, b)
        key = jnp.where(b >= 0x8000, 0xFFFF - b, b + 0x8000)
        key = jnp.where((b & 0x7FFF) > 0x7F80, 0, key)
        pos = lax.broadcasted_iota(I32, b.shape, 0) * T + lax.broadcasted_iota(I32, b.shape, 1)
        key = lax.bitcast_convert_type((key * S + (S - 1 - pos)) | (1 << 29), F32)
        sub = lax.broadcasted_iota(I32, (CAP, T), 0)
        top = jnp.zeros((CAP, T), F32)
        for c in range(CAP):
            mx = jnp.max(jnp.max(key, axis=0, keepdims=True), axis=1, keepdims=True)
            top = jnp.where(sub == c, mx, top)
            key = jnp.where(key == mx, 0.0, key)
        sel_ref[...] = lax.bitcast_convert_type(top, I32)

    def gather():
        top = sel_ref[...]
        key = (top & ((1 << 29) - 1)) // S
        b = jnp.where(key >= 0x8000, key - 0x8000, 0xFFFF - key)
        g = _rb(jax.nn.sigmoid(lax.bitcast_convert_type(b << 16, F32)))
        gate_ref[...] = jnp.concatenate([g] * (M // T), axis=1)
        sel = (S - 1) - (top & (S - 1))
        xn32 = xn_ref.bitcast(U32)
        xs = jnp.zeros((CAP, M), U32)
        sub = lax.broadcasted_iota(I32, (CAP, M), 0)
        for c in range(CAP):
            i = sel[c, 0]
            idx_ref[c] = i
            w = xn32[pl.ds(i >> 1, 1), :]
            xs = jnp.where(sub == c, (w >> ((i & 1) * 16).astype(U32)) << 16, xs)
        xs_ref[...] = lax.bitcast_convert_type(xs, F32)
        y_ref[...] = jnp.zeros((CAP, M), F32)

    def next_kv(j):
        xs = xs_ref[...].astype(BF16)
        y = y_ref[...]
        for n in range(2):
            f0 = (j - 1 + n) * T
            fs = pl.ds(pl.multiple_of(jnp.minimum(f0, F - T), T // 2), T)
            wk = [wk_b[0, h] if n == 0 else _half(wk_s[j + 2], h) for h in range(2)]
            wv = [_half(wv_s[j + 1 + n], h) for h in range(2)]
            k_ref[n, 0] = _dot(c_ref[...], wk[0]).astype(BF16)
            g = _rb(_dot_nt(xs, wg_ref[fs, :]))
            k_ref[n, 1] = _dot(c_ref[...], wk[1]).astype(BF16)
            u = _rb(_dot_nt(xs, wu_ref[fs, :]))
            v_ref[n, 0] = _dot(c_ref[...], wv[0]).astype(BF16)
            fresh = lax.broadcasted_iota(I32, (CAP, T), 1) >= f0 - (F - T)
            hid = jnp.where(fresh, _rb(g * jax.nn.sigmoid(g)) * u, 0.0).astype(BF16)
            y = y + _dot(hid, wd_ref[fs, :])
            v_ref[n, 1] = _dot(c_ref[...], wv[1]).astype(BF16)
        y_ref[...] = y

    def out_proj(j, n):
        rows = slice(OB[n], OB[n + 1])
        ctx = jnp.concatenate([ctx_ref[0, rows, :], ctx_ref[1, rows, :]], axis=1)
        a = acc_ref[rows, :] + _dot(ctx, wo_ref[j])
        acc_ref[rows, :] = a
        finish(rows, a)
        pl.when(j == HP - 1)(lambda: o_copy(n).start())

    def pair_body(j, carry):
        chk, big = carry
        odd = j & 1
        pl.when(j + 2 < HP)(lambda: start(w_copies(j + 2)))
        pl.when((odd == 1) & (j + 1 < HP))(lambda: wait(w_copies(j + 1)))
        pl.when(j == HP - 1)(scatter)

        for r0 in range(0, S, S // 2):
            rows = slice(r0, r0 + S // 2)
            for h in range(2):
                q_ref[h, rows, :] = (_dot(xn_ref[rows, :], wq_b[odd, h]) * qscale).astype(BF16)
        nxt = jnp.minimum(j + 1, HP - 1)
        nc = S // 2 // HP
        big = big | _big(wv_s[j]) | _big(c_ref.bitcast(U32)[pl.ds(pl.multiple_of(j * nc, nc), nc), :])
        top_tokens()

        tri = lax.broadcasted_iota(I32, (T, T), 1) <= lax.broadcasted_iota(I32, (T, T), 0)
        nt = BQ // T
        for qi in range(NQ):
            q0 = qi * BQ
            for h in range(2):
                q = q_ref[h, q0:q0 + BQ, :]
                ps = []
                for t in range(nt):
                    k0 = q0 + t * T
                    p = jnp.exp2(_dot_nt(q[t * T:], k_ref[odd, h, k0:k0 + T, :]))
                    pd = jnp.where(tri, p[:T], 0.0)
                    ps.append(jnp.concatenate([pd, p[T:]], axis=0) if t < nt - 1 else pd)
                accs, ls = [None] * nt, [None] * nt
                for t in range(nt):
                    k0 = q0 + t * T
                    o = _dot(ps[t].astype(BF16), v_ref[odd, h, k0:k0 + T, :])
                    for u in range(t, nt):
                        sl = slice((u - t) * T, (u - t + 1) * T)
                        ls[u] = ps[t][sl] if t == 0 else ls[u] + ps[t][sl]
                        accs[u] = o[sl] if t == 0 else accs[u] + o[sl]
                acc = jnp.concatenate(accs, axis=0)
                l = jnp.concatenate(ls, axis=0)
                for k0 in range(0, q0, BK):
                    p = jnp.exp2(_dot_nt(q, k_ref[odd, h, k0:k0 + BK, :]))
                    for t in range(0, BK, T):
                        l = l + p[:, t:t + T]
                    acc = acc + _dot(p.astype(BF16), v_ref[odd, h, k0:k0 + BK, :])
                l = jnp.sum(l, axis=1, keepdims=True)
                rl = pl.reciprocal(l, approx=True)
                rl = rl * (2.0 - l * rl)
                ctx_ref[h, q0:q0 + BQ, :] = (acc * rl).astype(BF16)
                chk = chk + jnp.sum((l + rl).reshape(-1, 8, 1), axis=0)
                if h == 0 and qi == 2:
                    out_proj(j, 0)
                    out_proj(j, 1)
        unpack(wq_s.at[nxt], wq_b.at[1 - odd])
        unpack(wk_s.at[nxt], wk_b.at[0])
        for n in range(2, len(OB) - 1):
            out_proj(j, n)

        @pl.when((odd == 1) & (j + 2 < HP))
        def _():
            wait(w_copies(j + 2))

            @pl.when(j == 1)
            def _():
                wait(ffn_copies)
                gather()
            next_kv(j)
        return chk, big

    chk, big = lax.fori_loop(0, HP, pair_body, (jnp.zeros((8, T), F32), jnp.zeros((8, T), U32)))
    unsafe = jnp.max(jnp.where((chk < SAFE) & (big == 0), 0.0, 1.0)) > 0.0
    out_copies = [o_copy(n) for n in range(len(OB) - 1)]
    wait(out_copies)

    @pl.when(unsafe)
    def _():
        def blocks(body):
            def step(i, _):
                body(i, pl.ds(pl.multiple_of(i * T, T), T))
                return 0
            lax.fori_loop(0, S // T, step, 0)

        def clear(i, rows):
            acc_ref[rows, :] = jnp.zeros((T, M), F32)
        blocks(clear)
        scatter()

        def pair(j, _):
            unpack(wq_s.at[j], wq_b.at[0])
            unpack(wk_s.at[j], wk_b.at[0])
            unpack(wv_s.at[j], wv_b.at[0])

            def head(h, _):
                def proj(i, rows):
                    k_ref[0, 0, rows, :] = _dot(c_ref[rows, :], wk_b[0, h]).astype(BF16)
                    v_ref[0, 0, rows, :] = _dot(c_ref[rows, :], wv_b[0, h]).astype(BF16)
                blocks(proj)

                def attend(i, rows):
                    q = (_dot(xn_ref[rows, :], wq_b[0, h]) * qscale).astype(BF16)
                    keep = (lax.broadcasted_iota(I32, (T, S), 1)
                            <= lax.broadcasted_iota(I32, (T, S), 0) + i * T)
                    s = jnp.where(keep, _dot_nt(q, k_ref[0, 0]), MASKED)
                    p = jnp.exp2(s - jnp.max(s, axis=1, keepdims=True))
                    p = p / jnp.sum(p, axis=1, keepdims=True)
                    ctx = _dot(p.astype(BF16), v_ref[0, 0]).astype(BF16)
                    wo = wo_ref[j, pl.ds(pl.multiple_of(h * D, D), D), :]
                    acc_ref[rows, :] += _dot(ctx, wo)
                blocks(attend)
                return 0
            lax.fori_loop(0, 2, head, 0)
            return 0
        lax.fori_loop(0, HP, pair, 0)

        blocks(lambda i, rows: finish(rows, acc_ref[rows, :]))
        start(out_copies)
        wait(out_copies)


@jax.jit
def pallas_parallel_sum__compressed_kv_cla__moe_arch_mod__prompt_kernel(
        A_x, A_c_kv, A_w_q, A_w_uk, A_w_uv, A_w_o, B_x, B_w_r, B_w_gate, B_w_up, B_w_down):
    _, S, M = A_x.shape
    DC = A_c_kv.shape[2]
    _, H, D = A_w_q.shape
    F = B_w_down.shape[0]
    HP = H // 2
    assert (S, H, D) == (OB[-1], 32, T) and (HP - 3) * T < F <= (HP - 2) * T and F % (T // 2) == 0
    vm, dma = pltpu.VMEM, pltpu.SemaphoreType.DMA
    hbm = pl.BlockSpec(memory_space=pl.ANY)
    out = pl.pallas_call(
        _kernel,
        out_shape=jax.ShapeDtypeStruct((S, M), BF16),
        in_specs=[hbm] * 6 + [pl.BlockSpec(memory_space=vm)] + [hbm] * 3,
        out_specs=hbm,
        scratch_shapes=[
            vm((S, M), BF16), vm((S, DC), BF16), vm((S, M), BF16), vm((S, M), F32), vm((S, M), BF16),
            vm((2, S, D), BF16), vm((2, 2, S, D), BF16), vm((2, 2, S, D), BF16), vm((2, S, D), BF16),
            vm((HP, M, D), U32), vm((HP, DC, D), U32), vm((HP, DC, D), U32), vm((HP, 2 * D, M), BF16),
            vm((2, 2, M, D), BF16), vm((2, 2, DC, D), BF16), vm((2, 2, DC, D), BF16),
            vm((F, M), BF16), vm((F, M), BF16), vm((F, M), BF16),
            vm((S // T, T), F32), vm((CAP, T), I32), vm((CAP, M), F32), vm((CAP, M), F32), vm((CAP, M), F32),
            pltpu.SMEM((CAP,), I32),
            dma((S // RB,)), dma((HP,)), dma((len(OB) - 1,)), dma((3,)),
        ],
        compiler_params=pltpu.CompilerParams(
            vmem_limit_bytes=100 * 1024 * 1024, disable_bounds_checks=True),
    )(A_x.reshape(S, M), A_c_kv.reshape(S, DC), A_w_q, A_w_uk, A_w_uv, A_w_o.reshape(HP, 2 * D, M),
      B_w_r, B_w_gate.T, B_w_up.T, B_w_down)
    return out.reshape(1, S, M)
```
